```python
import jax
import jax.numpy as jnp

def _softmax(x, axis=-1):
    return jax.nn.softmax(x, axis=axis)

def _gelu(x):
    return jax.nn.gelu(x, approximate=True)

def _silu(x):
    return jax.nn.silu(x)

def _sigmoid(x):
    return jax.nn.sigmoid(x)

def _layernorm(x, axis=-1, eps=1e-05):
    m = jnp.mean(x, axis=axis, keepdims=True)
    v = jnp.var(x, axis=axis, keepdims=True)
    return (x - m) / jnp.sqrt(v + eps)

def _scatter_add(tgt, idx, src, axis=0):
    return tgt.at[idx].add(src)

def _segment_sum(src, seg, n):
    return jax.ops.segment_sum(src, seg, n)

class _Rng:

    def __init__(self, key):
        self._k = key

    def _next(self):
        self._k, sub = jax.random.split(self._k)
        return sub

    def normal(self, shape):
        return jax.random.normal(self._next(), shape, dtype=jnp.bfloat16)

    def randint(self, lo, hi, shape):
        return jax.random.randint(self._next(), shape, lo, hi, dtype=jnp.int32)

    def uniform(self, shape, lo=0.0, hi=1.0):
        return jax.random.uniform(self._next(), shape, jnp.bfloat16, lo, hi)

    def permutation(self, n):
        return jax.random.permutation(self._next(), n)
kernel_name = 'standalone__dilated_atrous__vision'

def setup_inputs():
    _rng = _Rng(jax.random.key(int.from_bytes(__import__("os").urandom(4), "little")))
    _w = lambda a: (lambda t: t.astype(jnp.bfloat16) if jnp.issubdtype(t.dtype, jnp.floating) else t)(jnp.asarray(a))
    H = W = 384
    C = 384
    k = 1
    return {'x': _w((lambda *s: _rng.normal(s) * 0.05)(1, H, W, C)), 'w': _w((lambda *s: _rng.normal(s) * 0.05)(k, k, C, C) * (1.0 / (k * C ** 0.5)))}

def reference(x, w):
    B, H, W, C = x.shape
    k = 1
    rate = 2
    pad = (k - 1) * rate // 2
    xp = jnp.pad(x, ((0, 0), (pad, pad), (pad, pad), (0, 0)))
    out = jnp.zeros_like(x)
    for i in range(k):
        for j in range(k):
            tap = xp[:, i * rate:i * rate + H, j * rate:j * rate + W, :].copy()
            out = out + jnp.einsum('bhwc,co->bhwo', tap, w[i, j])
    return out
```

```python
import jax
import jax.numpy as jnp
from jax import lax
import jax.experimental.pallas as pl
import jax.experimental.pallas.tpu as pltpu

_STREAMS = 6
_SLAB_ROWS = 768
_SEG_ROWS = 48
_TAIL_ROWS = 96
_WRITE_RATE = 2


@jax.jit
def pallas_standalone__dilated_atrous__vision_kernel(
    x: jax.Array,
    w: jax.Array,
):
    B, H, W, C = x.shape
    assert w.shape == (1, 1, C, C)
    S, L, R, T = _STREAMS, _SLAB_ROWS, _SEG_ROWS, _TAIL_ROWS
    G = (B * H * W) // (S * L)
    assert G * S * L == B * H * W
    G0 = (9 * G + 15) // 16

    def kernel_function(x_hbm, w_hbm, o_hbm, buf, w_buf, read_sems, write_sem, aux_sems):
        def read_block(g):
            return pltpu.make_async_copy(x_hbm.at[g], buf.at[g], read_sems.at[g])

        read_w = pltpu.make_async_copy(w_hbm, w_buf, aux_sems.at[0])
        read_last_head = pltpu.make_async_copy(
            x_hbm.at[G - 1, :, pl.ds(0, L - T)], buf.at[G - 1, :, pl.ds(0, L - T)],
            read_sems.at[G - 1])
        read_last_tail = pltpu.make_async_copy(
            x_hbm.at[G - 1, :, pl.ds(L - T, T)], buf.at[G - 1, :, pl.ds(L - T, T)],
            aux_sems.at[1])

        def compute_block(g):
            acc = jnp.dot(buf[g].reshape(S * L, C), w_buf[...],
                          preferred_element_type=jnp.float32)
            buf[g] = acc.astype(buf.dtype).reshape(S, L, C)

        def write_blocks(lo, hi):
            @pl.loop(lo, hi)
            def _(g):
                @pl.loop(0, L // R)
                def _(j):
                    rows = pl.ds(pl.multiple_of(j * R, R), R)
                    pltpu.make_async_copy(
                        buf.at[g, :, rows], o_hbm.at[g, :, rows], write_sem).start()

        read_w.start()

        @pl.loop(0, G - 1)
        def _(g):
            read_block(g).start()

        read_last_head.start()
        read_last_tail.start()
        read_w.wait()

        @pl.loop(0, G0)
        def _(g):
            read_block(g).wait()
            compute_block(g)

        @pl.loop(G0, G - 1)
        def _(g):
            read_block(g).wait()

        read_last_head.wait()

        write_blocks(0, _WRITE_RATE)
        read_last_tail.wait()

        @pl.loop(G0, G)
        def _(g):
            compute_block(g)
            i = g - G0
            write_blocks(jnp.minimum(_WRITE_RATE * (i + 1), g),
                         jnp.minimum(_WRITE_RATE * (i + 2), g + 1))

        write_blocks(min(_WRITE_RATE * (G - G0 + 1), G), G)
        pltpu.make_async_copy(buf, o_hbm, write_sem).wait()

    out = pl.pallas_call(
        kernel_function,
        in_specs=[pl.BlockSpec(memory_space=pl.ANY), pl.BlockSpec(memory_space=pl.ANY)],
        out_specs=pl.BlockSpec(memory_space=pl.ANY),
        out_shape=jax.ShapeDtypeStruct((G, S, L, C), x.dtype),
        scratch_shapes=[
            pltpu.VMEM((G, S, L, C), x.dtype),
            pltpu.VMEM((C, C), w.dtype),
            pltpu.SemaphoreType.DMA((G,)),
            pltpu.SemaphoreType.DMA(()),
            pltpu.SemaphoreType.DMA((2,)),
        ],
        compiler_params=pltpu.CompilerParams(vmem_limit_bytes=124 * 1024 * 1024),
    )(x.reshape(G, S, L, C), w.reshape(C, C))
    return out.reshape(B, H, W, C)
```

```python
import jax
import jax.numpy as jnp
import jax.experimental.pallas as pl
import jax.experimental.pallas.tpu as pltpu

_STREAMS = 6
_STREAM_ROWS = 4096
_SEG_ROWS = 32
_BURST_ROWS = 512
_UNIT_ROWS = 256
_LEAD_BURSTS = 4
_TAIL_ROWS = 192
_FIRST_WRITES = 3
_WRITE_SKIP = 8


@jax.jit
def pallas_standalone__dilated_atrous__vision_kernel(
    x: jax.Array,
    w: jax.Array,
):
    B, H, W, C = x.shape
    assert w.shape == (1, 1, C, C)
    S, L = _STREAMS, _STREAM_ROWS
    G = (B * H * W) // (S * L)
    assert G * S * L == B * H * W and G % 2 == 0
    rows = G * L
    n_bursts = rows // _BURST_ROWS
    n_units = rows // _UNIT_ROWS
    units_per_burst = _BURST_ROWS // _UNIT_ROWS

    bounds = [0, _BURST_ROWS, 3 * _BURST_ROWS]
    bounds += [g * L for g in range(1, G // 2 + 1)]
    bounds += [rows - L, rows - _TAIL_ROWS, rows]
    n_early = bounds.index(rows // 2)
    n_ranges = len(bounds) - 1

    last_burst_unit = n_bursts - 1 - _LEAD_BURSTS
    read_units = last_burst_unit + 2
    assert read_units * _UNIT_ROWS <= rows // 2
    for k in range(n_early):
        assert (_LEAD_BURSTS + bounds[k] // _UNIT_ROWS + 1) * _BURST_ROWS >= bounds[k + 1]

    def writes_before(unit):
        done = unit - read_units
        return _FIRST_WRITES + done - done // _WRITE_SKIP

    for unit in range(read_units, n_units + 1):
        assert writes_before(unit) * units_per_burst <= unit

    def kernel_function(x_hbm, w_hbm, o_hbm, w_buf, buf, read_sems, write_sem, w_sem):
        def window(ref, index, size):
            start = pl.multiple_of((index % (L // size)) * size, size)
            return ref.at[index // (L // size), :, pl.ds(start, size)]

        def read_burst(burst, sem_of_segment):
            src, dst = window(x_hbm, burst, _BURST_ROWS), window(buf, burst, _BURST_ROWS)
            for seg in range(0, _BURST_ROWS, _SEG_ROWS):
                for queue in range(2):
                    part = (pl.ds(queue * (S // 2), S // 2), pl.ds(seg, _SEG_ROWS))
                    pltpu.make_async_copy(
                        src.at[part], dst.at[part], read_sems.at[sem_of_segment(seg)]
                    ).start(priority=queue)

        def read_regular_burst(burst):
            sem = jnp.int32(0)
            for bound in bounds[1:-2]:
                sem += (burst * _BURST_ROWS >= bound).astype(jnp.int32)
            read_burst(burst, lambda seg: sem)

        def read_last_burst():
            read_burst(
                n_bursts - 1,
                lambda seg: n_ranges - (2 if seg < _BURST_ROWS - _TAIL_ROWS else 1))

        def wait_reads(k):
            lo, hi = bounds[k], bounds[k + 1]
            if (hi - lo) % L == 0:
                region = (pl.ds(lo // L, (hi - lo) // L),)
            else:
                region = (lo // L, slice(None), pl.ds(lo % L, hi - lo))
            pltpu.make_async_copy(x_hbm.at[region], buf.at[region], read_sems.at[k]).wait()

        def write_burst(burst):
            src, dst = window(buf, burst, _BURST_ROWS), window(o_hbm, burst, _BURST_ROWS)
            for seg in range(0, _BURST_ROWS, _SEG_ROWS):
                part = (slice(None), pl.ds(seg, _SEG_ROWS))
                pltpu.make_async_copy(src.at[part], dst.at[part], write_sem).start(priority=1)

        def multiply(unit):
            tile = window(buf, unit, _UNIT_ROWS)
            acc = jnp.dot(tile[...].reshape(S * _UNIT_ROWS, C), w_buf[...],
                          preferred_element_type=jnp.float32)
            tile[...] = acc.astype(buf.dtype).reshape(S, _UNIT_ROWS, C)

        read_w = pltpu.make_async_copy(w_hbm, w_buf, w_sem)
        read_w.start()
        pl.loop(0, _LEAD_BURSTS)(read_regular_burst)
        read_w.wait()

        @pl.loop(0, read_units)
        def _(unit):
            pl.when(unit < last_burst_unit)(lambda: read_regular_burst(_LEAD_BURSTS + unit))
            pl.when(unit == last_burst_unit)(read_last_burst)
            for k in range(n_early):
                pl.when(unit * _UNIT_ROWS == bounds[k])(lambda k=k: wait_reads(k))
            multiply(unit)

        for k in range(n_early, n_ranges - 1):
            wait_reads(k)
        pl.loop(0, _FIRST_WRITES)(write_burst)
        wait_reads(n_ranges - 1)

        @pl.loop(read_units, n_units)
        def _(unit):
            multiply(unit)
            burst = writes_before(unit)
            pl.when(writes_before(unit + 1) > burst)(lambda: write_burst(burst))

        pl.loop(writes_before(n_units), n_bursts)(write_burst)
        pltpu.make_async_copy(buf, o_hbm, write_sem).wait()

    out = pl.pallas_call(
        kernel_function,
        in_specs=[pl.BlockSpec(memory_space=pl.ANY), pl.BlockSpec(memory_space=pl.ANY)],
        out_specs=pl.BlockSpec(memory_space=pl.ANY),
        out_shape=jax.ShapeDtypeStruct((G, S, L, C), x.dtype),
        scratch_shapes=[
            pltpu.VMEM((C, C), w.dtype),
            pltpu.VMEM((G, S, L, C), x.dtype),
            pltpu.SemaphoreType.DMA((n_ranges,)),
            pltpu.SemaphoreType.DMA(()),
            pltpu.SemaphoreType.DMA(()),
        ],
        compiler_params=pltpu.CompilerParams(vmem_limit_bytes=124 * 1024 * 1024),
    )(x.reshape(G, S, L, C), w.reshape(C, C))
    return out.reshape(B, H, W, C)
```

```python
import jax
import jax.numpy as jnp
import jax.experimental.pallas as pl
import jax.experimental.pallas.tpu as pltpu

_STREAMS = 6
_STREAM_ROWS = 4096
_SEG_ROWS = 32
_BURST_ROWS = 512
_UNIT_ROWS = 256
_LEAD_BURSTS = 4
_TAIL_ROWS = 192
_FIRST_WRITES = 3
_WRITE_SKIP = 8


@jax.jit
def pallas_standalone__dilated_atrous__vision_kernel(
    x: jax.Array,
    w: jax.Array,
):
    B, H, W, C = x.shape
    assert w.shape == (1, 1, C, C)
    S, L = _STREAMS, _STREAM_ROWS
    G = (B * H * W) // (S * L)
    assert G * S * L == B * H * W and G % 2 == 0
    rows = G * L
    n_bursts = rows // _BURST_ROWS
    n_units = rows // _UNIT_ROWS
    units_per_burst = _BURST_ROWS // _UNIT_ROWS

    bounds = [0, _BURST_ROWS, 3 * _BURST_ROWS]
    bounds += [g * L for g in range(1, G // 2 + 1)]
    bounds += [rows - L, rows - _TAIL_ROWS, rows]
    n_early = bounds.index(rows // 2)
    n_ranges = len(bounds) - 1

    last_burst_unit = n_bursts - 1 - _LEAD_BURSTS
    read_units = last_burst_unit + 2
    assert read_units * _UNIT_ROWS <= rows // 2
    for k in range(n_early):
        assert (_LEAD_BURSTS + bounds[k] // _UNIT_ROWS + 1) * _BURST_ROWS >= bounds[k + 1]

    def writes_before(unit):
        done = unit - read_units
        return _FIRST_WRITES + done - done // _WRITE_SKIP

    for unit in range(read_units, n_units + 1):
        assert writes_before(unit) * units_per_burst <= unit

    def kernel_function(x_hbm, w_hbm, o_hbm, w_buf, buf, read_sems, write_sem, w_sem):
        def window(ref, index, size):
            start = pl.multiple_of((index % (L // size)) * size, size)
            return ref.at[index // (L // size), :, pl.ds(start, size)]

        def read_burst(burst, sem_of_segment, queues=(0, 1)):
            src, dst = window(x_hbm, burst, _BURST_ROWS), window(buf, burst, _BURST_ROWS)
            for seg in range(0, _BURST_ROWS, _SEG_ROWS):
                for half, queue in enumerate(queues):
                    part = (pl.ds(half * (S // 2), S // 2), pl.ds(seg, _SEG_ROWS))
                    pltpu.make_async_copy(
                        src.at[part], dst.at[part], read_sems.at[sem_of_segment(seg)]
                    ).start(priority=queue)

        def read_first_burst():
            read_burst(0, lambda seg: 0, queues=(1, 1))

        def read_regular_burst(burst):
            sem = jnp.int32(0)
            for bound in bounds[1:-2]:
                sem += (burst * _BURST_ROWS >= bound).astype(jnp.int32)
            read_burst(burst, lambda seg: sem)

        def read_last_burst():
            read_burst(
                n_bursts - 1,
                lambda seg: n_ranges - (2 if seg < _BURST_ROWS - _TAIL_ROWS else 1))

        def wait_reads(k):
            lo, hi = bounds[k], bounds[k + 1]
            if (hi - lo) % L == 0:
                region = (pl.ds(lo // L, (hi - lo) // L),)
            else:
                region = (lo // L, slice(None), pl.ds(lo % L, hi - lo))
            pltpu.make_async_copy(x_hbm.at[region], buf.at[region], read_sems.at[k]).wait()

        def write_burst(burst):
            src, dst = window(buf, burst, _BURST_ROWS), window(o_hbm, burst, _BURST_ROWS)
            for seg in range(0, _BURST_ROWS, _SEG_ROWS):
                part = (slice(None), pl.ds(seg, _SEG_ROWS))
                pltpu.make_async_copy(src.at[part], dst.at[part], write_sem).start(priority=1)

        def multiply(unit):
            tile = window(buf, unit, _UNIT_ROWS)
            acc = jnp.dot(tile[...].reshape(S * _UNIT_ROWS, C), w_buf[...],
                          preferred_element_type=jnp.float32)
            tile[...] = acc.astype(buf.dtype).reshape(S, _UNIT_ROWS, C)

        read_w = pltpu.make_async_copy(w_hbm, w_buf, w_sem)
        read_w.start()
        read_first_burst()
        pl.loop(1, _LEAD_BURSTS)(read_regular_burst)
        read_w.wait()

        @pl.loop(0, read_units)
        def _(unit):
            pl.when(unit < last_burst_unit)(lambda: read_regular_burst(_LEAD_BURSTS + unit))
            pl.when(unit == last_burst_unit)(read_last_burst)
            for k in range(n_early):
                pl.when(unit * _UNIT_ROWS == bounds[k])(lambda k=k: wait_reads(k))
            multiply(unit)

        for k in range(n_early, n_ranges - 1):
            wait_reads(k)
        pl.loop(0, _FIRST_WRITES)(write_burst)
        wait_reads(n_ranges - 1)

        @pl.loop(read_units, n_units)
        def _(unit):
            multiply(unit)
            burst = writes_before(unit)
            pl.when(writes_before(unit + 1) > burst)(lambda: write_burst(burst))

        if writes_before(n_units) < n_bursts:
            pl.loop(writes_before(n_units), n_bursts)(write_burst)
        pltpu.make_async_copy(buf, o_hbm, write_sem).wait()

    out = pl.pallas_call(
        kernel_function,
        in_specs=[pl.BlockSpec(memory_space=pl.ANY), pl.BlockSpec(memory_space=pl.ANY)],
        out_specs=pl.BlockSpec(memory_space=pl.ANY),
        out_shape=jax.ShapeDtypeStruct((G, S, L, C), x.dtype),
        scratch_shapes=[
            pltpu.VMEM((C, C), w.dtype),
            pltpu.VMEM((G, S, L, C), x.dtype),
            pltpu.SemaphoreType.DMA((n_ranges,)),
            pltpu.SemaphoreType.DMA(()),
            pltpu.SemaphoreType.DMA(()),
        ],
        compiler_params=pltpu.CompilerParams(vmem_limit_bytes=124 * 1024 * 1024),
    )(x.reshape(G, S, L, C), w.reshape(C, C))
    return out.reshape(B, H, W, C)
```
